```python
import os as _os
_os.environ.setdefault("JAX_PLATFORMS", "cpu")
import jax
import jax.numpy as jnp

def _softmax(x, axis=-1):
    return jax.nn.softmax(x, axis=axis)
def _gelu(x):
    return jax.nn.gelu(x, approximate=True)
def _silu(x):
    return jax.nn.silu(x)
def _sigmoid(x):
    return jax.nn.sigmoid(x)
def _layernorm(x, axis=-1, eps=1e-5):
    m = jnp.mean(x, axis=axis, keepdims=True)
    v = jnp.var(x, axis=axis, keepdims=True)
    return (x - m) / jnp.sqrt(v + eps)
def _scatter_add(tgt, idx, src, axis=0):
    return tgt.at[idx].add(src)
def _segment_sum(src, seg, n):
    return jax.ops.segment_sum(src, seg, n)
class _Rng:
    def __init__(self, key):
        self._k = key
    def _next(self):
        self._k, sub = jax.random.split(self._k)
        return sub
    def normal(self, shape):
        return jax.random.normal(self._next(), shape, dtype=jnp.bfloat16)
    def randint(self, lo, hi, shape):
        return jax.random.randint(self._next(), shape, lo, hi, dtype=jnp.int32)
    def uniform(self, shape, lo=0.0, hi=1.0):
        return jax.random.uniform(self._next(), shape, jnp.bfloat16, lo, hi)
    def permutation(self, n):
        return jax.random.permutation(self._next(), n)


kernel_name = 'gated_mix__sliding_block__dense_activation_silu__prompt'

def setup_inputs():
    _rng = _Rng(jax.random.key(int.from_bytes(__import__("os").urandom(4), "little")))
    _w = (lambda a: (lambda t: t.astype(jnp.bfloat16) if jnp.issubdtype(t.dtype, jnp.floating) else t)(jnp.asarray(a)))
    def _A_setup():
        B, S, D = 1, 2048, 640
        return {
            "x": _w((lambda *s: _rng.normal(s) * 0.05)(B, S, D)),
            "wqkv": _w((lambda *s: _rng.normal(s) * 0.4)(D, 3 * D)),
            "wo": _w((lambda *s: _rng.normal(s) * 0.05)(D, D)),
        }
    _A_in = _A_setup()

    def _B_setup():
        B, S, D, F = 1, 2048, 640, 1536
        return {
            "x": _w((lambda *s: _rng.normal(s) * 0.05)(B, S, D)),
            "w1": _w((lambda *s: _rng.normal(s) * 1.6)(D, F) * (D ** -0.5)),
            "w2": _w((lambda *s: _rng.normal(s) * 1.6)(F, D) * (F ** -0.5)),
        }
    _B_in = _B_setup()

    return {
        "A_x": _A_in["x"],
        "A_wqkv": _A_in["wqkv"],
        "A_wo": _A_in["wo"],
        "B_x": _B_in["x"],
        "B_w1": _B_in["w1"],
        "B_w2": _B_in["w2"],
        "gate_w": _w((lambda *s: _rng.normal(s) * 0.05)(640) * 16.0),
    }

def reference(A_x, A_wqkv, A_wo, B_x, B_w1, B_w2, gate_w):
    def _A_ref(x, wqkv, wo):
        B, S, D = x.shape
        H = 32; Dh = D // H; W = 256
        qkv = (lambda x, *d: x.transpose(*d))((x @ wqkv).reshape(B, S, 3, H, Dh), 2, 0, 3, 1, 4)
        q, k, v = qkv[0], qkv[1], qkv[2]
        scores = jnp.einsum("bhqd,bhkd->bhqk", q, k) * (Dh ** -0.5)
        idx = jnp.arange(S)
        mask = (idx[:, None] - idx[None, :] >= 0) & (idx[:, None] - idx[None, :] < W)
        scores = jnp.where(mask[None, None], scores, -1e9)
        p = _softmax(scores, axis=-1)
        o = jnp.einsum("bhqk,bhkd->bhqd", p, v)
        return (lambda x, *d: x.transpose(*d))(o, 0, 2, 1, 3).reshape(B, S, D) @ wo

    def _B_ref(x, w1, w2):
        h = jnp.einsum("bsd,df->bsf", x, w1)
        h = _silu(h)
        out = jnp.einsum("bsf,fd->bsd", h, w2)
        return out

    x = A_x
    g = _sigmoid((x * gate_w).sum(-1, keepdims=True))
    a = _A_ref(x, A_wqkv, A_wo)
    b = _B_ref(x, B_w1, B_w2)
    return g * a + (1 - g) * b
```

```python
import functools

import jax
import jax.numpy as jnp
import numpy as np
from jax import lax
from jax.experimental import pallas as pl
from jax.experimental.pallas import tpu as pltpu

S, D, H, DH, W, F = 2048, 640, 32, 20, 256, 1536
T = 128
HT = T // 2
NT_DIMS = (((1,), (1,)), ((), ()))
LOG2E = 1.4426950408889634
G = 4
NG = H // G
BF = jnp.bfloat16
F32 = jnp.float32
U32 = jnp.uint32
NCH = D // 128


def _grp(g):
    lo = g * G * DH
    hi = lo + G * DH - 1
    return lo // 128, hi // 128, lo % 128


def _head_chunks(h):
    lo, hi = h * DH, h * DH + DH - 1
    return lo // 128, hi // 128


def _iota(shape, dim):
    return lax.broadcasted_iota(jnp.int32, shape, dim)


def make(BQ=256, flags=None, SCHED=0, ORDER=0):
    NQT = BQ // T
    NKT = (S + W) // T
    NS = S // BQ

    def kern(x_hbm, gw_hbm, wqkv_hbm, wo_hbm, w1_hbm, w2_hbm, o_ref,
             x_s, gw_s, wqk_s, wv_s, wo_s, w1_s, w2_s, sems, qsems, xsems,
             k_scr, vt_scr, wvt_scr, q_scr, ot_scr, h_scr, ob_scr, b_scr):
        step = pl.program_id(0)

        CW = 256
        NCW = 2 * D // CW

        def wdma(name, c=None):
            if name == "qk":
                cs = slice(c * CW, (c + 1) * CW)
                return pltpu.make_async_copy(wqkv_hbm.at[:, cs], wqk_s.at[:, cs], qsems.at[c])
            i, src, dst = {
                "v": (0, wqkv_hbm.at[:, 2 * D:3 * D], wv_s),
                "o": (1, wo_hbm, wo_s),
                "1": (2, w1_hbm, w1_s),
                "2": (3, w2_hbm, w2_s),
                "g": (4, gw_hbm, gw_s),
            }[name]
            return pltpu.make_async_copy(src, dst, sems.at[i])

        def xdma(blk):
            rows = pl.ds(pl.multiple_of(blk * BQ, BQ), BQ)
            return pltpu.make_async_copy(x_hbm.at[rows, :], x_s.at[rows, :], xsems.at[blk])

        def xrows(blk):
            return pl.ds(pl.multiple_of(blk * BQ, BQ), BQ)

        def proj_qk(blk, hook=None):
            kch = {}
            for c in range(NCW):
                if hook is not None:
                    hook(c)
                y = jnp.dot(x_s[xrows(blk), :], wqk_s[:, c * CW:(c + 1) * CW], preferred_element_type=F32)
                for s_ in range(CW // 128):
                    col = c * (CW // 128) + s_
                    ys_ = y[:, s_ * 128:(s_ + 1) * 128]
                    if col < NCH:
                        q_scr[xrows(blk), col * 128:(col + 1) * 128] = (ys_ * (DH ** -0.5 * LOG2E)).astype(BF)
                    else:
                        kch[col - NCH] = ys_.astype(BF)
            row0 = pl.multiple_of(blk * BQ + W, T)
            lane = _iota((BQ, 128), 1)
            for g in range(NG):
                c0, c1, a = _grp(g)
                kv = kch[c0] if c0 == c1 else jnp.where(lane >= a, kch[c0], kch[c1])
                k_scr[g, pl.ds(row0, BQ), :] = kv

        def proj_v(blk):
            x = x_s[xrows(blk), :]
            vt = lax.dot_general(wvt_scr[...], x, NT_DIMS, preferred_element_type=F32)
            rowi = _iota((32, BQ), 0)
            kt0 = blk * NQT + 2
            for h in range(H):
                w0 = (h * DH // 16) * 16
                off = h * DH - w0
                r1 = 0 if off == 12 else 31
                win = jnp.where(rowi == r1, 1.0, vt[w0:w0 + 32, :]).astype(BF)
                for t in range(NQT):
                    vt_scr[kt0 + t, h] = win[:, t * T:(t + 1) * T]

        def rest(blk, extra=()):
            i64 = _iota((HT, T), 0)
            q64 = _iota((HT, T), 1)
            mask_lo = i64 + HT > q64
            mask_hi = i64 <= q64
            i32 = _iota((HT // 2, T), 0)
            q32 = _iota((HT // 2, T), 1)

            def pk(c_even, c_odd):
                return (jnp.where(c_even, U32(0x0000FFFF), U32(0)) | jnp.where(c_odd, U32(0xFFFF0000), U32(0)))

            mlo_u = pk(2 * i32 + HT > q32, 2 * i32 + 1 + HT > q32)
            mhi_u = pk(2 * i32 <= q32, 2 * i32 + 1 <= q32)
            sub8 = _iota((8, T), 0)
            lane_q = _iota((T // 2, 128), 1)
            lane_e = _iota((HT // 2, 128), 1)

            def lmask(lo, hi):
                return jnp.where((lane_q >= lo) & (lane_q < hi), U32(0xFFFFFFFF), U32(0))

            def in_head(lane, h):
                lo = (h * DH) % 128
                hi = lo + DH
                if hi <= 128:
                    return (lane >= lo) & (lane < hi)
                return (lane >= lo) | (lane < hi - 128)

            def qmask(t, h):
                c0, c1 = _head_chunks(h)
                lo = h * DH
                qrows = pl.ds(pl.multiple_of(blk * BQ + t * T, T), T)
                a0 = lo - c0 * 128
                q0 = pltpu.bitcast(q_scr[qrows, c0 * 128:(c0 + 1) * 128], U32)
                if c0 == c1:
                    return q0 & lmask(a0, a0 + DH)
                a1 = lo + DH - c1 * 128
                q1 = pltpu.bitcast(q_scr[qrows, c1 * 128:(c1 + 1) * 128], U32)
                return (q0 & lmask(a0, 128)) | (q1 & lmask(0, a1))

            def stage_a(t, g):
                qm = [qmask(t, g * G + j) for j in range(G)]
                q0 = pl.multiple_of(blk * BQ + t * T, T)
                ka = pltpu.bitcast(k_scr[g, pl.ds(q0, HT), :], U32)
                kb = pltpu.bitcast(k_scr[g, pl.ds(pl.multiple_of(q0 + 5 * HT, HT), HT), :], U32)
                sel = in_head(lane_e, g * G) | in_head(lane_e, g * G + 2)
                l1 = pltpu.bitcast(jnp.where(sel, ka, kb), BF)
                l2 = pltpu.bitcast(jnp.where(sel, kb, ka), BF)
                ha = [m[0:HT // 2] for m in qm]
                hb = [m[HT // 2:HT] for m in qm]
                src1 = pltpu.bitcast(jnp.concatenate([ha[0], hb[1], ha[2], hb[3]], axis=0), BF)
                src2 = pltpu.bitcast(jnp.concatenate([ha[1], hb[0], ha[3], hb[2]], axis=0), BF)
                e1 = lax.dot_general(l1, src1, NT_DIMS, preferred_element_type=F32)
                e2 = lax.dot_general(l2, src2, NT_DIMS, preferred_element_type=F32)
                srcm = pltpu.bitcast(jnp.concatenate(qm, axis=0), BF)
                km = k_scr[g, pl.ds(pl.multiple_of(q0 + HT, HT), 2 * T), :]
                s = lax.dot_general(km, srcm, NT_DIMS, preferred_element_type=F32)
                xs = [e1[:, 0:T], e2[:, 0:T], e1[:, T:2 * T], e2[:, T:2 * T]]
                ys = [e2[:, 0:T], e1[:, 0:T], e2[:, T:2 * T], e1[:, T:2 * T]]
                res = []
                for j in range(G):
                    sj = s[:, j * T:(j + 1) * T]
                    lo = jnp.where(mask_lo, sj[0:HT], ys[j])
                    mid = sj[HT:3 * HT]
                    hi = jnp.where(mask_hi, sj[3 * HT:4 * HT], xs[j])
                    m = jnp.max(jnp.maximum(jnp.maximum(lo, hi), jnp.maximum(mid[0:HT], mid[HT:T])),
                                axis=0, keepdims=True)
                    res.append((lo, mid, hi, m))
                return res

            def stage_b(t, g, res):
                kt = blk * NQT + t
                outs = []
                for j in range(G):
                    h = g * G + j
                    lo, mid, hi, m = res[j]
                    plo = jnp.exp2(lo - m)
                    pmid = jnp.exp2(mid - m)
                    phi = jnp.exp2(hi - m)
                    a_ = jnp.where(mask_hi, phi, 0.0)
                    b_ = jnp.where(mask_lo, plo, 0.0)
                    p = jnp.concatenate([phi - a_, b_, pmid, a_, plo - b_], axis=0).astype(BF)
                    v = jnp.concatenate([vt_scr[kt, h], vt_scr[kt + 1, h], vt_scr[kt + 2, h]], axis=1)
                    o = jnp.dot(v, p, preferred_element_type=F32)
                    off = h * DH % 16
                    r1 = 0 if off == 12 else 31
                    inv = 1.0 / o[r1:r1 + 1, :]
                    outs.append((o, inv, off))
                cs = slice(t * T, (t + 1) * T)
                for jj in range(G // 2):
                    oe, ie, offe = outs[2 * jj]
                    oo, io, offo = outs[2 * jj + 1]
                    r = (g * G + 2 * jj) * DH
                    ot_scr[r:r + 16, cs] = oe[offe:offe + 16] * ie
                    ot_scr[r + 16:r + 24, cs] = jnp.where(sub8 < 4, oe[offe + 16:offe + 24] * ie,
                                                          oo[offo - 4:offo + 4] * io)
                    ot_scr[r + 24:r + 40, cs] = oo[offo + 4:offo + 20] * io

            def xblk():
                return x_s[xrows(blk), :]

            def ffn1(c, wd=128):
                hh = jnp.dot(xblk(), w1_s[:, c * wd:(c + 1) * wd], preferred_element_type=F32)
                u = 0.5 * hh
                h_scr[:, c * wd:(c + 1) * wd] = (u + u * jnp.tanh(u)).astype(BF)

            def ffn2(n):
                b_scr[:, n * 128:(n + 1) * 128] = jnp.dot(h_scr[...], w2_s[:, n * 128:(n + 1) * 128],
                                                          preferred_element_type=F32)

            def otr(t):
                ob_scr[t * T:(t + 1) * T, :] = ot_scr[:, t * T:(t + 1) * T].astype(BF).T

            def gate():
                return jax.nn.sigmoid(jnp.sum(xblk().astype(F32) * gw_s[...].astype(F32)[None, :], axis=-1, keepdims=True))

            def mix(n, gt):
                cs = slice(n * 128, (n + 1) * 128)
                a = jnp.dot(ob_scr[...], wo_s[:, cs], preferred_element_type=F32)
                o_ref[:, cs] = (gt * a + (1.0 - gt) * b_scr[:, cs]).astype(o_ref.dtype)

            units = [(t, g) for t in range(NQT) for g in range(NG)]
            nu = len(units)
            fill = [functools.partial(ffn1, c) for c in range(F // 128)]
            fill += [functools.partial(ffn2, n) for n in range(NCH)]
            slots = [[] for _ in range(nu + 1)]
            if SCHED == 0:
                for i, f in enumerate(fill):
                    slots[min(i, nu)].append(f)
            elif SCHED == 1:
                per = len(fill) / (nu + 1)
                for i, f in enumerate(fill):
                    slots[min(int(i / per), nu)].append(f)
            for t in range(NQT - 1):
                slots[(t + 1) * NG + 1].insert(0, functools.partial(otr, t))
            nxt = stage_a(*units[0])
            for i, u in enumerate(units):
                cur = nxt
                if i + 1 < nu:
                    nxt = stage_a(*units[i + 1])
                if ORDER == 0:
                    for f in slots[i]:
                        f()
                    stage_b(*u, cur)
                else:
                    stage_b(*u, cur)
                    for f in slots[i]:
                        f()
            otr(NQT - 1)
            for f in slots[nu]:
                f()
            gt = gate()
            extra = list(extra)
            for n in range(NCH):
                mix(n, gt)
                if n == 1 and extra:
                    extra.pop(0)()
            for f in extra:
                f()

        @pl.when(step == 0)
        def _():
            xdma(0).start()
            wdma("qk", 0).start()
            wdma("qk", 1).start()
            vt_scr[0:2] = jnp.zeros((2, H, 32, T), BF)

            def hook(c):
                if c == 0:
                    xdma(0).wait()
                wdma("qk", c).wait()
                if c + 2 < NCW:
                    wdma("qk", c + 2).start()
                if c == 2:
                    xdma(1).start()
                if c == 3:
                    wdma("v").start()
                if c == 4:
                    xdma(2).start()
                    wdma("1").start()
            proj_qk(0, hook)
            for g in range(NG):
                k0 = k_scr[g, W:W + 16, :]
                k_scr[g, 0:W, :] = jnp.broadcast_to(k0[0:1, :], (W, 128))
            xdma(1).wait()
            proj_qk(1)
            xdma(2).wait()
            wdma("2").start()
            wdma("o").start()
            wdma("g").start()
            proj_qk(2)
            wdma("v").wait()
            wvt_scr[...] = wv_s[...].T
            proj_v(0)
            proj_v(1)
            proj_v(2)
            wdma("1").wait()
            wdma("2").wait()
            wdma("o").wait()
            wdma("g").wait()
            for b in range(3, NS):
                xdma(b).start()

        @pl.when((step > 0) & (step < NS - 2))
        def _():
            xdma(step + 2).wait()
            rest(step - 1, [functools.partial(proj_qk, step + 2), functools.partial(proj_v, step + 2)])

        @pl.when(step >= NS - 2)
        def _():
            rest(step - 1)

    any_spec = pl.BlockSpec(memory_space=pl.ANY)
    return pl.pallas_call(
        kern, grid=(NS + 1,),
        in_specs=[any_spec] * 6,
        out_specs=pl.BlockSpec((BQ, D), lambda i: (jnp.maximum(i - 1, 0), 0)),
        out_shape=jax.ShapeDtypeStruct((S, D), BF),
        scratch_shapes=[
            pltpu.VMEM((S, D), BF), pltpu.VMEM((D,), BF),
            pltpu.VMEM((D, 2 * D), BF), pltpu.VMEM((D, D), BF), pltpu.VMEM((D, D), BF),
            pltpu.VMEM((D, F), BF), pltpu.VMEM((F, D), BF),
            pltpu.SemaphoreType.DMA((5,)), pltpu.SemaphoreType.DMA((5,)), pltpu.SemaphoreType.DMA((NS,)),
            pltpu.VMEM((NG, S + W, 128), BF),
            pltpu.VMEM((NKT, H, 32, T), BF),
            pltpu.VMEM((D, D), BF),
            pltpu.VMEM((S, D), BF),
            pltpu.VMEM((D, BQ), F32),
            pltpu.VMEM((BQ, F), BF),
            pltpu.VMEM((BQ, D), BF),
            pltpu.VMEM((BQ, D), F32),
        ],
        compiler_params=pltpu.CompilerParams(dimension_semantics=("arbitrary",),
                                             vmem_limit_bytes=100 * 1024 * 1024, flags=flags),
        name="fused")


@jax.jit
def pallas_gated_mix__sliding_block__dense_activation_silu__prompt_kernel(
    A_x: jax.Array,
    A_wqkv: jax.Array,
    A_wo: jax.Array,
    B_x: jax.Array,
    B_w1: jax.Array,
    B_w2: jax.Array,
    gate_w: jax.Array,
):
    del B_x
    out = make()(A_x.reshape(S, D), gate_w, A_wqkv, A_wo, B_w1, B_w2)
    return out.reshape(1, S, D)
```

```python
import functools

import jax
import jax.numpy as jnp
import numpy as np
from jax import lax
from jax.experimental import pallas as pl
from jax.experimental.pallas import tpu as pltpu

S, D, H, DH, W, F = 2048, 640, 32, 20, 256, 1536
T = 128
HT = T // 2
NT_DIMS = (((1,), (1,)), ((), ()))
LOG2E = 1.4426950408889634
G = 4
NG = H // G
BF = jnp.bfloat16
F32 = jnp.float32
U32 = jnp.uint32
NCH = D // 128


def _grp(g):
    lo = g * G * DH
    hi = lo + G * DH - 1
    return lo // 128, hi // 128, lo % 128


def _head_chunks(h):
    lo, hi = h * DH, h * DH + DH - 1
    return lo // 128, hi // 128


def _iota(shape, dim):
    return lax.broadcasted_iota(jnp.int32, shape, dim)


MID0 = "a0|a1|a2|a3|a4|a5|a6|a7|a8|o0 a9|a10|a11|b0|b1|b2|b3|o1 b4 m0 m1 q0 q1 q2 q3 q4 m2 m3 m4 v0 v1"
LAST0 = "a0|a1|a2|a3|a4|a5|a6|a7|a8|o0 a9|a10|a11|b0|b1|b2|b3|o1 b4 m0 m1 m2 m3 m4"
MULT = [1, 5, 3]
M256 = "a0||a1||a2||a3||a4|o0|a5||b0|b1|b2|b3|o1 b4 m0 m1 q0 q1 q2 q3 q4 m2 m3 m4 v0 v1"
L256 = "a0||a1||a2||a3||a4|o0|a5||b0|b1|b2|b3|o1 b4 m0 m1 m2 m3 m4"
M256b = "a0|a1|a2|a3|a4|a5|b0||b1|o0|b2||b3||b4||o1 m0 m1 q0 q1 q2 q3 q4 m2 m3 m4 v0 v1"
L256b = "a0|a1|a2|a3|a4|a5|b0||b1|o0|b2||b3||b4||o1 m0 m1 m2 m3 m4"
M0c = "a0|a1|a2|a3|a4|a5|a6|a7|a8|o0 a9|a10|a11|b0|b1|b2|b3|o1 b4 q0 m0 q1 m1 q2 m2 q3 m3 q4 m4 v0 v1"
M0d = "a0|a1|a2|a3|a4|a5|a6|a7|a8|o0 a9|a10|a11|b0|b1|b2|b3|q0 o1 b4 q1 m0 q2 m1 q3 m2 q4 m3 v0 m4 v1"
L0d = "a0 a1|a2|a3|a4|a5|a6|a7|a8|a9|o0 a10|a11|b0|b1|b2|b3|b4|o1 m0 m1 m2 m3 m4"
M0e = "a0|a1|a2|a3|a4|a5|a6|a7|a8|o0 a9|a10|a11|b0|b1|b2|b3|q0 o1 q1 b4 q2 m0 q3 m1 q4 m2 m3 v0 m4 v1"
M0f = "a0|a1|a2|a3|a4|a5|a6|a7|o0 a8|a9|a10|a11|b0|b1|b2|b3|q0 o1 b4 m0 q1 m1 q2 m2 q3 m3 q4 m4 v0 v1"
M0g = "a0|a1|a2|a3|a4|a5|a6|a7|a8|o0 a9|a10|a11|b0|b1|b2|b3 |v0 o1 b4 m0 v1 m1 q0 m2 q1 m3 q2 m4 q3 q4"
M256c = "a0||a1||a2||a3||a4|o0|a5||b0|b1|b2|b3|q0 o1 b4 q1 m0 q2 m1 q3 m2 q4 m3 v0 m4 v1"
L256c = "a0||a1||a2||a3||a4|o0|a5|b0|b1|b2|b3|b4|o1 m0 m1 m2 m3 m4"
L0e = "a0|a1|a2|a3|a4|a5|a6|a7|a8|o0 a9|a10|a11 b0|b1|b2|b3|b4|o1 m0 m1 m2 m3 m4"
M256d = "a0||a1||a2||a3||a4|o0|a5||b0||b1||q0 o1 b2 q1 m0 q2 m1 q3 m2 q4 m3 v0 m4 v1"
M256e = "a0||a1||a2||a3|a4|a5|o0|b0||b1||b2||q0 o1 q1 m0 q2 m1 q3 m2 q4 m3 v0 m4 v1"
M256f = "|a0||a1||a2||a3||o0 a4||a5|b0|b1|b2|b3|q0 o1 b4 q1 m0 q2 m1 q3 m2 q4 m3 v0 m4 v1"
M256g = "a0||a1||a2||a3||a4|o0|a5||b0|b1|b2|b3 |v0 o1 b4 m0 v1 m1 q0 m2 q1 m3 q2 m4 q3 q4"
L256d = "a0||a1||a2||a3||a4|o0|a5|b0|b1|b2|b3||o1 b4 m0 m1 m2 m3 m4"
L256e = "a0||a1||a2||a3||a4|o0|a5||b0|b1|b2|b3|o1 b4 m0 m1 m2 m3 m4"
L0f = "a0|a1|a2|a3|a4|a5|a6|a7|a8|o0 a9|a10|a11|b0|b1|b2|b3|b4 o1 m0 m1 m2 m3 m4"
M256h = "a0||a1||a2||a3||a4|o0|a5||b0|b1|b2|b3|q0 o1 b4 q1 m0 q2 q3 m1 q4 m2 v0 v1"
M256i = "a0||a1||a2||a3||a4|o0|a5||b0|b1|b2|b3|q0 o1 b4 q1 q2 m0 q3 q4 v0 v1"
M512a = "a0|||a1||||a2||o0|||b0|b1|b2|b3|q0 o1 b4 q1 m0 q2 m1 q3 m2 q4 m3 v0 m4 v1"
M512b = "|a0||||a1|||o0|a2|||b0|b1|b2|b3|q0 o1 b4 q1 m0 q2 m1 q3 m2 q4 m3 v0 m4 v1"
L256h = "a0||a1||a2||a3||a4|o0|a5||b0|b1|b2|b3|o1 b4 m0 m1 m2"
L0h = "a0|a1|a2|a3|a4|a5|a6|a7|a8|o0 a9|a10|a11|b0|b1|b2|b3|o1 b4 m0 m1 m2"
L0i = "a0|a1|a2|a3|a4|a5|a6|a7|a8|o0 a9|a10|a11|b0|b1|b2|b3|o1 b4 m0"
L512a = "a0|||a1||||a2||o0|||b0|b1|b2|b3|o1 b4 m0 m1 m2 m3 m4"
MID1 = "a0 a1|a2 a3|a4 a5|a6 a7|a8 a9|a10 a11|q0|q1|q2|o0 q3|q4|b0|b1|b2|b3|b4|o1 v0 m0 m1 m2 m3 m4 v1"
MID2 = "a0 q0|a1 a2|a3 q1|a4 a5|a6 q2|a7 a8|a9 q3|a10 a11|q4|o0 b0|b1|b2|b3|b4|v0|v1|o1 m0 m1 m2 m3 m4"
LAST1 = "a0 a1|a2|a3 a4|a5|a6 a7|a8|a9 a10|a11|b0|o0|b1|b2|b3|b4|||o1 m0 m1 m2 m3 m4"


def make(BQ=256, flags=None, PLAN_MID=MID0, PLAN_LAST=LAST0, F1WM=128, F1WL=128, F2WM=128, F2WL=128, WVEARLY=1, MWM=128, MWL=128):
    NQT = BQ // T
    NKT = (S + W) // T
    NS = S // BQ

    def kern(x_hbm, gw_hbm, wqkv_hbm, wo_hbm, w1_hbm, w2_hbm, o_ref,
             x_s, gw_s, wqk_s, wv_s, wo_s, w1_s, w2_s, sems, qsems, xsems,
             k_scr, vt_scr, wvt_scr, q_scr, ot_scr, h_scr, ob_scr, b_scr):
        step = pl.program_id(0)

        CW = 256
        NCW = 2 * D // CW

        def wdma(name, c=None):
            if name == "qk":
                cs = slice(c * CW, (c + 1) * CW)
                return pltpu.make_async_copy(wqkv_hbm.at[:, cs], wqk_s.at[:, cs], qsems.at[c])
            i, src, dst = {
                "v": (0, wqkv_hbm.at[:, 2 * D:3 * D], wv_s),
                "o": (1, wo_hbm, wo_s),
                "1": (2, w1_hbm, w1_s),
                "2": (3, w2_hbm, w2_s),
                "g": (4, gw_hbm, gw_s),
            }[name]
            return pltpu.make_async_copy(src, dst, sems.at[i])

        def xdma(blk):
            rows = pl.ds(pl.multiple_of(blk * BQ, BQ), BQ)
            return pltpu.make_async_copy(x_hbm.at[rows, :], x_s.at[rows, :], xsems.at[blk])

        def xrows(blk):
            return pl.ds(pl.multiple_of(blk * BQ, BQ), BQ)

        def proj_qk_tasks(blk, hook=None, nb=1):
            kch = {}
            NR = nb * BQ

            def xrows(b):
                return pl.ds(pl.multiple_of(b * BQ, BQ), NR)

            def task(c):
                if hook is not None:
                    hook(c)
                y = jnp.dot(x_s[xrows(blk), :], wqk_s[:, c * CW:(c + 1) * CW], preferred_element_type=F32)
                row0 = pl.multiple_of(blk * BQ + W, T)
                lane = _iota((NR, 128), 1)
                for s_ in range(CW // 128):
                    col = c * (CW // 128) + s_
                    ys_ = y[:, s_ * 128:(s_ + 1) * 128]
                    if col < NCH:
                        q_scr[xrows(blk), col * 128:(col + 1) * 128] = (ys_ * (DH ** -0.5 * LOG2E)).astype(BF)
                    else:
                        kc = col - NCH
                        kch[kc] = ys_.astype(BF)
                        for g in range(NG):
                            c0, c1, a = _grp(g)
                            if c1 == kc:
                                kv = kch[c0] if c0 == c1 else jnp.where(lane >= a, kch[c0], kch[c1])
                                k_scr[g, pl.ds(row0, NR), :] = kv
            return [functools.partial(task, c) for c in range(NCW)]

        def proj_v_tasks(blk):
            def task(t):
                rows = pl.ds(pl.multiple_of(blk * BQ + t * T, T), T)
                vt = lax.dot_general(wvt_scr[...], x_s[rows, :], NT_DIMS, preferred_element_type=F32)
                rowi = _iota((32, T), 0)
                kt = blk * NQT + 2 + t
                for h in range(H):
                    w0 = (h * DH // 16) * 16
                    off = h * DH - w0
                    r1 = 0 if off == 12 else 31
                    vt_scr[kt, h] = jnp.where(rowi == r1, 1.0, vt[w0:w0 + 32, :]).astype(BF)
            return [functools.partial(task, t) for t in range(NQT)]

        def proj_qk(blk, hook=None, nb=1):
            for f in proj_qk_tasks(blk, hook, nb):
                f()

        def proj_v(blk):
            for f in proj_v_tasks(blk):
                f()

        def rest(blk, nblk=None):
            F1W = F1WM if nblk is not None else F1WL
            F2W = F2WM if nblk is not None else F2WL
            MW = MWM if nblk is not None else MWL
            i64 = _iota((HT, T), 0)
            q64 = _iota((HT, T), 1)
            mask_lo = i64 + HT > q64
            mask_hi = i64 <= q64
            nmask_lo = i64 + HT <= q64
            nmask_hi = i64 > q64
            sub8 = _iota((8, T), 0)
            lane_q = _iota((T // 2, 128), 1)
            lane_e = _iota((HT // 2, 128), 1)

            def lmask(lo, hi):
                return jnp.where((lane_q >= lo) & (lane_q < hi), U32(0xFFFFFFFF), U32(0))

            def in_head(lane, h):
                lo = (h * DH) % 128
                hi = lo + DH
                if hi <= 128:
                    return (lane >= lo) & (lane < hi)
                return (lane >= lo) | (lane < hi - 128)

            def qmask(t, h):
                c0, c1 = _head_chunks(h)
                lo = h * DH
                qrows = pl.ds(pl.multiple_of(blk * BQ + t * T, T), T)
                a0 = lo - c0 * 128
                q0 = pltpu.bitcast(q_scr[qrows, c0 * 128:(c0 + 1) * 128], U32)
                if c0 == c1:
                    return q0 & lmask(a0, a0 + DH)
                a1 = lo + DH - c1 * 128
                q1 = pltpu.bitcast(q_scr[qrows, c1 * 128:(c1 + 1) * 128], U32)
                return (q0 & lmask(a0, 128)) | (q1 & lmask(0, a1))

            def stage_a(t, g):
                qm = [qmask(t, g * G + j) for j in range(G)]
                q0 = pl.multiple_of(blk * BQ + t * T, T)
                ka = pltpu.bitcast(k_scr[g, pl.ds(q0, HT), :], U32)
                kb = pltpu.bitcast(k_scr[g, pl.ds(pl.multiple_of(q0 + 5 * HT, HT), HT), :], U32)
                sel = in_head(lane_e, g * G) | in_head(lane_e, g * G + 2)
                l1 = pltpu.bitcast(jnp.where(sel, ka, kb), BF)
                l2 = pltpu.bitcast(jnp.where(sel, kb, ka), BF)
                ha = [m[0:HT // 2] for m in qm]
                hb = [m[HT // 2:HT] for m in qm]
                src1 = pltpu.bitcast(jnp.concatenate([ha[0], hb[1], ha[2], hb[3]], axis=0), BF)
                src2 = pltpu.bitcast(jnp.concatenate([ha[1], hb[0], ha[3], hb[2]], axis=0), BF)
                e1 = lax.dot_general(l1, src1, NT_DIMS, preferred_element_type=F32)
                e2 = lax.dot_general(l2, src2, NT_DIMS, preferred_element_type=F32)
                srcm = pltpu.bitcast(jnp.concatenate(qm, axis=0), BF)
                km = k_scr[g, pl.ds(pl.multiple_of(q0 + HT, HT), 2 * T), :]
                s = lax.dot_general(km, srcm, NT_DIMS, preferred_element_type=F32)
                xs = [e1[:, 0:T], e2[:, 0:T], e1[:, T:2 * T], e2[:, T:2 * T]]
                ys = [e2[:, 0:T], e1[:, 0:T], e2[:, T:2 * T], e1[:, T:2 * T]]
                res = []
                for j in range(G):
                    sj = s[:, j * T:(j + 1) * T]
                    lo = jnp.where(mask_lo, sj[0:HT], ys[j])
                    mid = sj[HT:3 * HT]
                    hi = jnp.where(mask_hi, sj[3 * HT:4 * HT], xs[j])
                    m = jnp.max(jnp.maximum(jnp.maximum(lo, hi), jnp.maximum(mid[0:HT], mid[HT:T])),
                                axis=0, keepdims=True)
                    res.append((lo, mid, hi, m))
                return res

            def stage_b(t, g, res):
                kt = blk * NQT + t
                outs = []
                for j in range(G):
                    h = g * G + j
                    lo, mid, hi, m = res[j]
                    plo = jnp.exp2(lo - m)
                    pmid = jnp.exp2(mid - m)
                    phi = jnp.exp2(hi - m)
                    p = jnp.concatenate([jnp.where(nmask_hi, phi, 0.0), jnp.where(mask_lo, plo, 0.0), pmid,
                                         jnp.where(mask_hi, phi, 0.0), jnp.where(nmask_lo, plo, 0.0)],
                                        axis=0).astype(BF)
                    v = jnp.concatenate([vt_scr[kt, h], vt_scr[kt + 1, h], vt_scr[kt + 2, h]], axis=1)
                    o = jnp.dot(v, p, preferred_element_type=F32)
                    off = h * DH % 16
                    r1 = 0 if off == 12 else 31
                    inv = 1.0 / o[r1:r1 + 1, :]
                    outs.append((o, inv, off))
                cs = slice(t * T, (t + 1) * T)
                for jj in range(G // 2):
                    oe, ie, offe = outs[2 * jj]
                    oo, io, offo = outs[2 * jj + 1]
                    r = (g * G + 2 * jj) * DH
                    ot_scr[r:r + 16, cs] = oe[offe:offe + 16] * ie
                    ot_scr[r + 16:r + 24, cs] = jnp.where(sub8 < 4, oe[offe + 16:offe + 24] * ie,
                                                          oo[offo - 4:offo + 4] * io)
                    ot_scr[r + 24:r + 40, cs] = oo[offo + 4:offo + 20] * io

            def xblk():
                return x_s[xrows(blk), :]

            def ffn1(c, wd=128):
                hh = jnp.dot(xblk(), w1_s[:, c * wd:(c + 1) * wd], preferred_element_type=F32)
                u = 0.5 * hh
                h_scr[:, c * wd:(c + 1) * wd] = (u + u * jnp.tanh(u)).astype(BF)

            def ffn2(n):
                cs = slice(n * F2W, min((n + 1) * F2W, D))
                b_scr[:, cs] = jnp.dot(h_scr[...], w2_s[:, cs], preferred_element_type=F32)

            def otr(t):
                ob_scr[t * T:(t + 1) * T, :] = ot_scr[:, t * T:(t + 1) * T].astype(BF).T

            def gate():
                return jax.nn.sigmoid(jnp.sum(xblk().astype(F32) * gw_s[...].astype(F32)[None, :], axis=-1, keepdims=True))

            def mix(n, gt):
                cs = slice(n * MW, min((n + 1) * MW, D))
                a = jnp.dot(ob_scr[...], wo_s[:, cs], preferred_element_type=F32)
                o_ref[:, cs] = (gt * a + (1.0 - gt) * b_scr[:, cs]).astype(o_ref.dtype)

            units = [(t, g) for t in range(NQT) for g in range(NG)]
            nu = len(units)
            tasks = {}
            for c in range(F // F1W):
                tasks[f"a{c}"] = functools.partial(ffn1, c, F1W)
            for n in range(-(-D // F2W)):
                tasks[f"b{n}"] = functools.partial(ffn2, n)
            for t in range(NQT):
                tasks[f"o{t}"] = functools.partial(otr, t)
            if nblk is not None:
                for c, f in enumerate(proj_qk_tasks(nblk)):
                    tasks[f"q{c}"] = f
                for c, f in enumerate(proj_v_tasks(nblk)):
                    tasks[f"v{c}"] = f
            gt = [None]

            def mixn(n):
                if gt[0] is None:
                    gt[0] = gate()
                mix(n, gt[0])
            for n in range(-(-D // MW)):
                tasks[f"m{n}"] = functools.partial(mixn, n)
            plan = (PLAN_MID if nblk is not None else PLAN_LAST).split("|")
            assert len(plan) == nu + 1, len(plan)
            used = [w for p_ in plan for w in p_.split()]
            assert sorted(used) == sorted(tasks), (sorted(used), sorted(tasks))
            nxt = stage_a(*units[0])
            for i, u in enumerate(units):
                cur = nxt
                if i + 1 < nu:
                    nxt = stage_a(*units[i + 1])
                for w in plan[i].split():
                    tasks[w]()
                stage_b(*u, cur)
            for w in plan[nu].split():
                tasks[w]()

        @pl.when(step == 0)
        def _():
            xdma(0).start()
            wdma("qk", 0).start()
            wdma("qk", 1).start()
            vt_scr[0:2] = jnp.zeros((2, H, 32, T), BF)

            def hook(c):
                if c == 0:
                    xdma(0).wait()
                wdma("qk", c).wait()
                if c + 2 < NCW:
                    wdma("qk", c + 2).start()
                if c == 2:
                    xdma(1).start()
                if c == 3:
                    wdma("v").start()
                if c == 4:
                    xdma(2).start()
            proj_qk(0, hook)
            wdma("1").start()
            for g in range(NG):
                k0 = k_scr[g, W:W + 16, :]
                k_scr[g, 0:W, :] = jnp.broadcast_to(k0[0:1, :], (W, 128))
            xdma(1).wait()
            proj_qk(1)
            wdma("2").start()
            xdma(2).wait()
            wdma("v").wait()
            wvt_scr[...] = wv_s[...].T
            proj_qk(2)
            wdma("o").start()
            wdma("g").start()
            xdma(3).start()
            proj_v(0)
            proj_v(1)
            proj_v(2)
            wdma("1").wait()
            wdma("2").wait()
            wdma("o").wait()
            wdma("g").wait()

        @pl.when((step > 0) & (step < NS - 2))
        def _():
            @pl.when(step + 3 < NS)
            def _():
                xdma(step + 3).start()
            xdma(step + 2).wait()
            rest(step - 1, step + 2)

        @pl.when(step >= NS - 2)
        def _():
            rest(step - 1)

    any_spec = pl.BlockSpec(memory_space=pl.ANY)
    return pl.pallas_call(
        kern, grid=(NS + 1,),
        in_specs=[any_spec] * 6,
        out_specs=pl.BlockSpec((BQ, D), lambda i: (jnp.maximum(i - 1, 0), 0)),
        out_shape=jax.ShapeDtypeStruct((S, D), BF),
        scratch_shapes=[
            pltpu.VMEM((S, D), BF), pltpu.VMEM((D,), BF),
            pltpu.VMEM((D, 2 * D), BF), pltpu.VMEM((D, D), BF), pltpu.VMEM((D, D), BF),
            pltpu.VMEM((D, F), BF), pltpu.VMEM((F, D), BF),
            pltpu.SemaphoreType.DMA((5,)), pltpu.SemaphoreType.DMA((5,)), pltpu.SemaphoreType.DMA((NS,)),
            pltpu.VMEM((NG, S + W, 128), BF),
            pltpu.VMEM((NKT, H, 32, T), BF),
            pltpu.VMEM((D, D), BF),
            pltpu.VMEM((S, D), BF),
            pltpu.VMEM((D, BQ), F32),
            pltpu.VMEM((BQ, F), BF),
            pltpu.VMEM((BQ, D), BF),
            pltpu.VMEM((BQ, D), F32),
        ],
        compiler_params=pltpu.CompilerParams(dimension_semantics=("arbitrary",),
                                             vmem_limit_bytes=100 * 1024 * 1024, flags=flags),
        name="fused")


@jax.jit
def pallas_gated_mix__sliding_block__dense_activation_silu__prompt_kernel(
    A_x: jax.Array,
    A_wqkv: jax.Array,
    A_wo: jax.Array,
    B_x: jax.Array,
    B_w1: jax.Array,
    B_w2: jax.Array,
    gate_w: jax.Array,
):
    del B_x
    out = make(PLAN_MID=M256c, F1WM=256)(A_x.reshape(S, D), gate_w, A_wqkv, A_wo, B_w1, B_w2)
    return out.reshape(1, S, D)
```

```python
import functools

import jax
import jax.numpy as jnp
from jax import lax
from jax.experimental import pallas as pl
from jax.experimental.pallas import tpu as pltpu

S, D, H, DH, W, F = 2048, 640, 32, 20, 256, 1536
BQ = 256
T = 128
HT = T // 2
G = 4
NG = H // G
NQT = BQ // T
NKT = (S + W) // T
NS = S // BQ
NCH = D // 128
CW = 256
NCW = 2 * D // CW
BF = jnp.bfloat16
F32 = jnp.float32
U32 = jnp.uint32
NT_DIMS = (((1,), (1,)), ((), ()))
QSCALE = DH ** -0.5 * 1.4426950408889634

PLAN_MID = "a0||a1||a2||a3||a4|o0|a5||b0|b1|b2|b3|q0 o1 b4 q1 m0 q2 m1 q3 m2 q4 m3 v0 m4 v1"
PLAN_LAST = "a0|a1 a2||a3|a4||a5|a7|a6 a10 a8|a9||a11 o0|b0|b1|b2|b3|o1 b4 m1 m2 m0 m4 m3"
F1W_MID, F1W_LAST = 256, 128


def _group_chunks(g):
    lo = g * G * DH
    return lo // 128, (lo + G * DH - 1) // 128, lo % 128


def _head_chunks(h):
    return h * DH // 128, (h * DH + DH - 1) // 128


def _ones_row(h):
    return 0 if h * DH % 16 == 12 else 31


def _iota(shape, dim):
    return lax.broadcasted_iota(jnp.int32, shape, dim)


def _kernel(x_hbm, gw_hbm, wqkv_hbm, wo_hbm, w1_hbm, w2_hbm, o_ref,
            x_s, gw_s, wqk_s, wv_s, wo_s, w1_s, w2_s, wsems, qksems, xsems,
            k_s, vt_s, wvt_s, q_s, ot_s, h_s, ob_s, b_s):
    step = pl.program_id(0)

    def rows(blk):
        return pl.ds(pl.multiple_of(blk * BQ, BQ), BQ)

    def x_dma(blk):
        return pltpu.make_async_copy(x_hbm.at[rows(blk), :], x_s.at[rows(blk), :], xsems.at[blk])

    def qk_dma(c):
        cs = slice(c * CW, (c + 1) * CW)
        return pltpu.make_async_copy(wqkv_hbm.at[:, cs], wqk_s.at[:, cs], qksems.at[c])

    def w_dma(name):
        i, src, dst = {
            "v": (0, wqkv_hbm.at[:, 2 * D:3 * D], wv_s),
            "o": (1, wo_hbm, wo_s),
            "1": (2, w1_hbm, w1_s),
            "2": (3, w2_hbm, w2_s),
            "g": (4, gw_hbm, gw_s),
        }[name]
        return pltpu.make_async_copy(src, dst, wsems.at[i])

    def proj_qk_tasks(blk, hook=None):
        kch = {}

        def task(c):
            if hook is not None:
                hook(c)
            y = jnp.dot(x_s[rows(blk), :], wqk_s[:, c * CW:(c + 1) * CW], preferred_element_type=F32)
            krows = pl.ds(pl.multiple_of(blk * BQ + W, T), BQ)
            lane = _iota((BQ, 128), 1)
            for i in range(CW // 128):
                col = c * (CW // 128) + i
                yc = y[:, i * 128:(i + 1) * 128]
                if col < NCH:
                    q_s[rows(blk), col * 128:(col + 1) * 128] = (yc * QSCALE).astype(BF)
                    continue
                kch[col - NCH] = yc.astype(BF)
                for g in range(NG):
                    c0, c1, a = _group_chunks(g)
                    if c1 == col - NCH:
                        k_s[g, krows, :] = kch[c0] if c0 == c1 else jnp.where(lane >= a, kch[c0], kch[c1])

        return [functools.partial(task, c) for c in range(NCW)]

    def proj_v_tasks(blk):
        def task(t):
            xr = pl.ds(pl.multiple_of(blk * BQ + t * T, T), T)
            vt = lax.dot_general(wvt_s[...], x_s[xr, :], NT_DIMS, preferred_element_type=F32)
            row = _iota((32, T), 0)
            kt = blk * NQT + W // T + t
            for h in range(H):
                w0 = h * DH // 16 * 16
                vt_s[kt, h] = jnp.where(row == _ones_row(h), 1.0, vt[w0:w0 + 32, :]).astype(BF)

        return [functools.partial(task, t) for t in range(NQT)]

    def run(tasks):
        for f in tasks:
            f()

    def block_out(blk, nblk=None):
        f1w = F1W_MID if nblk is not None else F1W_LAST
        i64, q64 = _iota((HT, T), 0), _iota((HT, T), 1)
        lo_main, lo_edge = i64 + HT > q64, i64 + HT <= q64
        hi_main, hi_edge = i64 <= q64, i64 > q64
        sub8 = _iota((8, T), 0)
        lane_q = _iota((T // 2, 128), 1)
        lane_e = _iota((HT // 2, 128), 1)

        def lanes(lo, hi):
            return jnp.where((lane_q >= lo) & (lane_q < hi), U32(0xFFFFFFFF), U32(0))

        def in_head(lane, h):
            lo = h * DH % 128
            if lo + DH <= 128:
                return (lane >= lo) & (lane < lo + DH)
            return (lane >= lo) | (lane < lo + DH - 128)

        def q_head(t, h):
            c0, c1 = _head_chunks(h)
            qr = pl.ds(pl.multiple_of(blk * BQ + t * T, T), T)
            a0 = h * DH - c0 * 128
            q0 = pltpu.bitcast(q_s[qr, c0 * 128:(c0 + 1) * 128], U32)
            if c0 == c1:
                return q0 & lanes(a0, a0 + DH)
            q1 = pltpu.bitcast(q_s[qr, c1 * 128:(c1 + 1) * 128], U32)
            return (q0 & lanes(a0, 128)) | (q1 & lanes(0, a0 + DH - 128))

        def scores(t, g):
            qm = [q_head(t, g * G + j) for j in range(G)]
            r0 = pl.multiple_of(blk * BQ + t * T, T)
            ka = pltpu.bitcast(k_s[g, pl.ds(r0, HT), :], U32)
            kb = pltpu.bitcast(k_s[g, pl.ds(pl.multiple_of(r0 + 5 * HT, HT), HT), :], U32)
            even = in_head(lane_e, g * G) | in_head(lane_e, g * G + 2)
            k02 = pltpu.bitcast(jnp.where(even, ka, kb), BF)
            k13 = pltpu.bitcast(jnp.where(even, kb, ka), BF)
            qa = [m[0:HT // 2] for m in qm]
            qb = [m[HT // 2:HT] for m in qm]
            e1 = lax.dot_general(k02, pltpu.bitcast(jnp.concatenate([qa[0], qb[1], qa[2], qb[3]], axis=0), BF),
                                 NT_DIMS, preferred_element_type=F32)
            e2 = lax.dot_general(k13, pltpu.bitcast(jnp.concatenate([qa[1], qb[0], qa[3], qb[2]], axis=0), BF),
                                 NT_DIMS, preferred_element_type=F32)
            km = k_s[g, pl.ds(pl.multiple_of(r0 + HT, HT), 2 * T), :]
            s = lax.dot_general(km, pltpu.bitcast(jnp.concatenate(qm, axis=0), BF), NT_DIMS,
                                preferred_element_type=F32)
            first = [e1[:, 0:T], e2[:, 0:T], e1[:, T:2 * T], e2[:, T:2 * T]]
            final = [e2[:, 0:T], e1[:, 0:T], e2[:, T:2 * T], e1[:, T:2 * T]]
            res = []
            for j in range(G):
                sj = s[:, j * T:(j + 1) * T]
                lo = jnp.where(lo_main, sj[0:HT], final[j])
                mid = sj[HT:3 * HT]
                hi = jnp.where(hi_main, sj[3 * HT:4 * HT], first[j])
                m = jnp.max(jnp.maximum(jnp.maximum(lo, hi), jnp.maximum(mid[0:HT], mid[HT:T])),
                            axis=0, keepdims=True)
                res.append((lo, mid, hi, m))
            return res

        def attend(t, g, res):
            kt = blk * NQT + t
            outs = []
            for j in range(G):
                h = g * G + j
                lo, mid, hi, m = res[j]
                plo = jnp.exp2(lo - m)
                pmid = jnp.exp2(mid - m)
                phi = jnp.exp2(hi - m)
                p = jnp.concatenate([jnp.where(hi_edge, phi, 0.0), jnp.where(lo_main, plo, 0.0), pmid,
                                     jnp.where(hi_main, phi, 0.0), jnp.where(lo_edge, plo, 0.0)],
                                    axis=0).astype(BF)
                v = jnp.concatenate([vt_s[kt, h], vt_s[kt + 1, h], vt_s[kt + 2, h]], axis=1)
                o = jnp.dot(v, p, preferred_element_type=F32)
                r1 = _ones_row(h)
                outs.append((o, 1.0 / o[r1:r1 + 1, :], h * DH % 16))
            cs = slice(t * T, (t + 1) * T)
            for j in range(0, G, 2):
                (oe, ie, fe), (oo, io, fo) = outs[j], outs[j + 1]
                r = (g * G + j) * DH
                ot_s[r:r + 16, cs] = oe[fe:fe + 16] * ie
                ot_s[r + 16:r + 24, cs] = jnp.where(sub8 < 4, oe[fe + 16:fe + 24] * ie, oo[fo - 4:fo + 4] * io)
                ot_s[r + 24:r + 40, cs] = oo[fo + 4:fo + 20] * io

        def ffn_up(c):
            cs = slice(c * f1w, (c + 1) * f1w)
            u = 0.5 * jnp.dot(x_s[rows(blk), :], w1_s[:, cs], preferred_element_type=F32)
            h_s[:, cs] = (u + u * jnp.tanh(u)).astype(BF)

        def ffn_down(n):
            cs = slice(n * 128, (n + 1) * 128)
            b_s[:, cs] = jnp.dot(h_s[...], w2_s[:, cs], preferred_element_type=F32)

        def transpose_out(t):
            ob_s[t * T:(t + 1) * T, :] = ot_s[:, t * T:(t + 1) * T].astype(BF).T

        gate = []

        def mix(n):
            if not gate:
                xg = x_s[rows(blk), :].astype(F32) * gw_s[...].astype(F32)[None, :]
                gate.append(jax.nn.sigmoid(jnp.sum(xg, axis=-1, keepdims=True)))
            cs = slice(n * 128, (n + 1) * 128)
            a = jnp.dot(ob_s[...], wo_s[:, cs], preferred_element_type=F32)
            o_ref[:, cs] = (gate[0] * a + (1.0 - gate[0]) * b_s[:, cs]).astype(o_ref.dtype)

        tasks = {f"a{c}": functools.partial(ffn_up, c) for c in range(F // f1w)}
        tasks.update({f"b{n}": functools.partial(ffn_down, n) for n in range(NCH)})
        tasks.update({f"o{t}": functools.partial(transpose_out, t) for t in range(NQT)})
        tasks.update({f"m{n}": functools.partial(mix, n) for n in range(NCH)})
        if nblk is not None:
            tasks.update({f"q{c}": f for c, f in enumerate(proj_qk_tasks(nblk))})
            tasks.update({f"v{c}": f for c, f in enumerate(proj_v_tasks(nblk))})
        plan = [slot.split() for slot in (PLAN_MID if nblk is not None else PLAN_LAST).split("|")]
        units = [(t, g) for t in range(NQT) for g in range(NG)]
        assert len(plan) == len(units) + 1 and sorted(w for slot in plan for w in slot) == sorted(tasks)

        nxt = scores(*units[0])
        for i, unit in enumerate(units):
            cur = nxt
            if i + 1 < len(units):
                nxt = scores(*units[i + 1])
            run(tasks[w] for w in plan[i])
            attend(*unit, cur)
        run(tasks[w] for w in plan[-1])

    @pl.when(step == 0)
    def _():
        x_dma(0).start()
        qk_dma(0).start()
        qk_dma(1).start()
        vt_s[0:W // T] = jnp.zeros((W // T, H, 32, T), BF)

        def hook(c):
            if c == 0:
                x_dma(0).wait()
            qk_dma(c).wait()
            if c + 2 < NCW:
                qk_dma(c + 2).start()
            if c == 2:
                x_dma(1).start()
            if c == 3:
                w_dma("v").start()
            if c == 4:
                x_dma(2).start()

        run(proj_qk_tasks(0, hook))
        w_dma("1").start()
        for g in range(NG):
            k_s[g, 0:W, :] = jnp.broadcast_to(k_s[g, W:W + 16, :][0:1, :], (W, 128))
        x_dma(1).wait()
        run(proj_qk_tasks(1))
        w_dma("2").start()
        x_dma(2).wait()
        w_dma("v").wait()
        wvt_s[...] = wv_s[...].T
        run(proj_qk_tasks(2))
        w_dma("o").start()
        w_dma("g").start()
        x_dma(3).start()
        for b in range(3):
            run(proj_v_tasks(b))
        w_dma("1").wait()
        w_dma("2").wait()
        w_dma("o").wait()
        w_dma("g").wait()

    @pl.when((step > 0) & (step < NS - 2))
    def _():
        @pl.when(step + 3 < NS)
        def _():
            x_dma(step + 3).start()

        x_dma(step + 2).wait()
        block_out(step - 1, step + 2)

    @pl.when(step >= NS - 2)
    def _():
        block_out(step - 1)


@jax.jit
def pallas_gated_mix__sliding_block__dense_activation_silu__prompt_kernel(
    A_x: jax.Array,
    A_wqkv: jax.Array,
    A_wo: jax.Array,
    B_x: jax.Array,
    B_w1: jax.Array,
    B_w2: jax.Array,
    gate_w: jax.Array,
):
    del B_x
    any_spec = pl.BlockSpec(memory_space=pl.ANY)
    out = pl.pallas_call(
        _kernel,
        grid=(NS + 1,),
        in_specs=[any_spec] * 6,
        out_specs=pl.BlockSpec((BQ, D), lambda i: (jnp.maximum(i - 1, 0), 0)),
        out_shape=jax.ShapeDtypeStruct((S, D), BF),
        scratch_shapes=[
            pltpu.VMEM((S, D), BF),
            pltpu.VMEM((D,), BF),
            pltpu.VMEM((D, 2 * D), BF),
            pltpu.VMEM((D, D), BF),
            pltpu.VMEM((D, D), BF),
            pltpu.VMEM((D, F), BF),
            pltpu.VMEM((F, D), BF),
            pltpu.SemaphoreType.DMA((5,)),
            pltpu.SemaphoreType.DMA((NCW,)),
            pltpu.SemaphoreType.DMA((NS,)),
            pltpu.VMEM((NG, S + W, 128), BF),
            pltpu.VMEM((NKT, H, 32, T), BF),
            pltpu.VMEM((D, D), BF),
            pltpu.VMEM((S, D), BF),
            pltpu.VMEM((D, BQ), F32),
            pltpu.VMEM((BQ, F), BF),
            pltpu.VMEM((BQ, D), BF),
            pltpu.VMEM((BQ, D), F32),
        ],
        compiler_params=pltpu.CompilerParams(
            dimension_semantics=("arbitrary",), vmem_limit_bytes=100 * 1024 * 1024),
        name="gated_mix_swa_ffn",
    )(A_x.reshape(S, D), gate_w, A_wqkv, A_wo, B_w1, B_w2)
    return out.reshape(1, S, D)
```
